```python
import jax
import jax.numpy as jnp

def _softmax(x, axis=-1):
    return jax.nn.softmax(x, axis=axis)
def _gelu(x):
    return jax.nn.gelu(x, approximate=True)
def _silu(x):
    return jax.nn.silu(x)
def _sigmoid(x):
    return jax.nn.sigmoid(x)
def _layernorm(x, axis=-1, eps=1e-5):
    m = jnp.mean(x, axis=axis, keepdims=True)
    v = jnp.var(x, axis=axis, keepdims=True)
    return (x - m) / jnp.sqrt(v + eps)
def _scatter_add(tgt, idx, src, axis=0):
    return tgt.at[idx].add(src)
def _segment_sum(src, seg, n):
    return jax.ops.segment_sum(src, seg, n)
class _Rng:
    def __init__(self, key):
        self._k = key
    def _next(self):
        self._k, sub = jax.random.split(self._k)
        return sub
    def normal(self, shape):
        return jax.random.normal(self._next(), shape, dtype=jnp.bfloat16)
    def randint(self, lo, hi, shape):
        return jax.random.randint(self._next(), shape, lo, hi, dtype=jnp.int32)
    def uniform(self, shape, lo=0.0, hi=1.0):
        return jax.random.uniform(self._next(), shape, jnp.bfloat16, lo, hi)
    def permutation(self, n):
        return jax.random.permutation(self._next(), n)


kernel_name = 'parallel_sum__ssm_conv_h3__dense_activation_gelu__prompt'

def setup_inputs():
    _rng = _Rng(jax.random.key(int.from_bytes(__import__("os").urandom(4), "little")))
    _w = (lambda a: (lambda t: t.astype(jnp.bfloat16) if jnp.issubdtype(t.dtype, jnp.floating) else t)(jnp.asarray(a)))
    def _A_setup():
        B, S, D = 1, 2048, 640
        ks = 4
        return {
            "q": _w((lambda *s: _rng.normal(s) * 0.05)(B, S, D)),
            "k": _w((lambda *s: _rng.normal(s) * 0.05)(B, S, D)),
            "v": _w((lambda *s: _rng.normal(s) * 0.05)(B, S, D)),
            "shift_k": _w((lambda *s: _rng.normal(s) * 0.05)(D, ks) * 0.5),
            "ssm_k": _w((lambda *s: _rng.normal(s) * 0.05)(D, S) * (1.0 / S ** 0.5)),
            "ssm_D": _w((lambda *s: _rng.normal(s) * 0.05)(D)),
        }
    _A_in = _A_setup()

    def _B_setup():
        B, S, D, F = 1, 2048, 640, 1728
        return {
            "x": _w((lambda *s: _rng.normal(s) * 0.05)(B, S, D)),
            "w1": _w((lambda *s: _rng.normal(s) * 0.05)(D, F) * (D ** -0.5)),
            "b1": _w((lambda *s: _rng.normal(s) * 0.05)(F) * 0.01),
            "w2": _w((lambda *s: _rng.normal(s) * 0.05)(F, D) * (F ** -0.5)),
            "b2": _w((lambda *s: _rng.normal(s) * 0.05)(D) * 0.01),
        }
    _B_in = _B_setup()

    return {
        "A_q": _A_in["q"],
        "A_k": _A_in["k"],
        "A_v": _A_in["v"],
        "A_shift_k": _A_in["shift_k"],
        "A_ssm_k": _A_in["ssm_k"],
        "A_ssm_D": _A_in["ssm_D"],
        "B_x": _B_in["x"],
        "B_w1": _B_in["w1"],
        "B_b1": _B_in["b1"],
        "B_w2": _B_in["w2"],
        "B_b2": _B_in["b2"],
    }

def reference(A_q, A_k, A_v, A_shift_k, A_ssm_k, A_ssm_D, B_x, B_w1, B_b1, B_w2, B_b2):
    def _A_ref(q, k, v, shift_k, ssm_k, ssm_D):
        B, S, D = q.shape
        ks = shift_k.shape[-1]
        k_pad = jnp.pad(k, ((0, 0), (ks - 1, 0), (0, 0)))
        k_shift = jnp.zeros_like(k)
        for t in range(ks):
            k_shift = k_shift + k_pad[:, t:t + S, :] * shift_k[:, ks - 1 - t][None, None, :]
        kv = k_shift * v
        L = 2 * S
        kv_pad = jnp.pad(kv, ((0, 0), (0, S), (0, 0)))
        kf_pad = jnp.pad(ssm_k, ((0, 0), (0, S)))
        kv_f = (lambda x, axes=(-2,-1): jnp.fft.rfft2(x.astype(jnp.float32), axes=axes))(kv_pad[:, None, :, :], axes=(1, 2))
        kf_f = (lambda x, axes=(-2,-1): jnp.fft.rfft2(x.astype(jnp.float32), axes=axes))(kf_pad[:, None, :], axes=(1, 2))
        kf_f = (lambda x, *d: x.transpose(*d))(kf_f, 1, 2, 0)
        y_f = kv_f * kf_f[None, :, :, :]
        y = (lambda x, s, axes=(-2,-1): jnp.fft.irfft2(x, s=s, axes=axes).astype(jnp.bfloat16))(y_f, (1, L), axes=(1, 2))[:, 0, :S, :]
        y = y + kv * ssm_D[None, None, :]
        return q * y

    def _B_ref(x, w1, b1, w2, b2):
        h = jnp.einsum("bsd,df->bsf", x, w1) + b1
        h = _gelu(h)
        return jnp.einsum("bsf,fd->bsd", h, w2) + b2

    x = A_q
    xn = _layernorm(x, axis=-1)
    return x + _A_ref(xn, A_k, A_v, A_shift_k, A_ssm_k, A_ssm_D) + _B_ref(xn, B_w1, B_b1, B_w2, B_b2)
```

```python
import math

import jax
import jax.numpy as jnp
import numpy as np
import jax.experimental.pallas as pl
import jax.experimental.pallas.tpu as pltpu

T = 128
L = 128
UA, UB, UC = 2, 2, 4
GR, LR = 64, 32
G0, G1, HL, XL = 0.15, 0.85, 1.0, 3.0
L0, L1 = 0.0, 0.7


def _dft_consts():
    k = np.concatenate([np.arange(0, T, 2), np.arange(1, T, 2)])
    n = np.arange(T)
    ang = np.pi * (2 * k[:, None] + 1) * n[None, :] / (2 * T)
    fwd = np.concatenate([np.cos(ang), -np.sin(ang)], 0)
    inv = np.concatenate([np.cos(ang).T, -np.sin(ang).T], 1) / T
    perm = (np.arange(T) // 16) * 16 + (np.arange(T) % 8) * 2 + (np.arange(T) // 8) % 2
    fwd = np.concatenate([fwd, fwd[:, perm]], 0)
    return fwd.astype(np.float32), inv.astype(np.float32)


_FWD, _INV = _dft_consts()
_NT = (((1,), (1,)), ((), ()))


def _kernel(q_hbm, k_hbm, v_hbm, sk_ref, h_hbm, d_ref, w1_hbm, b1_ref, w2_hbm, b2_ref,
            f_ref, g_ref, o_hbm,
            q_s, k_s, v_s, h_s, w1_s, w2_s, xn0_s, xn1_s, kv0, kv1, kv2, kv3, kv4, act_s, xc_s, gc_s, hp_s, mlp_s, o_s,
            sq, sk, sv, sh, sw, so):
    _, S, D = q_hbm.shape
    F = w1_hbm.shape[0]
    NB = S // T
    NL = D // L
    NF = pl.cdiv(F, L)
    TA = UA * T
    NA = NB // UA
    f32, bf16, u32 = jnp.float32, jnp.bfloat16, jnp.uint32

    def rows_of(start, n):
        return pl.ds(pl.multiple_of(start, 16), n)

    def lanes(l):
        return pl.ds(l * L, L)

    def pk(b, off, n):
        return pl.ds(pl.multiple_of(b * (T // 2) + off // 2, 8), n // 2)

    def ld(ref, b, off, n):
        return pltpu.bitcast(ref[pk(b, off, n), :], bf16)

    def q_cp(i):
        return pltpu.make_async_copy(q_hbm.at[0, rows_of(i * TA, TA)], q_s.at[rows_of(i * TA, TA)], sq.at[i])

    def k_cp(i, l):
        return pltpu.make_async_copy(k_hbm.at[0, rows_of(i * TA, TA), lanes(l)],
                                     k_s.bitcast(bf16).at[rows_of(i * TA + l * (S + 16) + 16, TA)], sk.at[i])

    def v_cp(i):
        return pltpu.make_async_copy(v_hbm.at[0, rows_of(i * TA, TA)],
                                     v_s.bitcast(bf16).at[rows_of(i * TA, TA)], sv.at[i])

    def h_cp(i):
        return pltpu.make_async_copy(h_hbm.at[:, pl.ds(pl.multiple_of(i * TA, TA), TA)], h_s.at[i], sh.at[i])

    def o_cp(i):
        return pltpu.make_async_copy(o_s.at[rows_of(i * T, T)], o_hbm.at[0, rows_of(i * T, T)], so.at[i])

    def w_cp(w_hbm, w_s, l, s):
        return pltpu.make_async_copy(w_hbm.at[:, lanes(l)], w_s.bitcast(bf16).at[pl.ds(l * F, F)], sw.at[s])

    def start_kvh(i):
        for l in range(NL):
            k_cp(i, l).start()
        v_cp(i).start()
        h_cp(i).start()

    q_cp(0).start()
    for l in range(NL):
        w_cp(w1_hbm, w1_s, l, 0).start()
    start_kvh(0)
    q_cp(1).start()

    for l in range(NL):
        k_s[pk(0, l * (S + 16), 16), :] = jnp.zeros((8, L), u32)
    hp_s[...] = jnp.zeros(hp_s.shape, f32)
    skt = sk_ref[...].astype(f32)
    b1 = b1_ref[...].astype(f32).reshape(1, F)
    b2 = b2_ref[...].astype(f32).reshape(1, D)
    dd = d_ref[...].astype(f32).reshape(1, D)
    c1 = math.sqrt(2.0 / math.pi)
    c2 = c1 * 0.044715

    xn_s = (xn0_s, xn1_s)
    kv_s = (kv0, kv1, kv2, kv3, kv4)

    def layernorm(b, par, r0, n):
        x = q_s[rows_of(b * T + r0, n), :].astype(f32)
        m = jnp.mean(x, axis=-1, keepdims=True)
        xc = x - m
        var = jnp.mean(xc * xc, axis=-1, keepdims=True)
        xn = (xc * jax.lax.rsqrt(var + 1e-5)).astype(bf16)
        for l in range(NL):
            xn_s[par][pk(b, l * S + r0, n), :] = pltpu.bitcast(xn[:, l * L:(l + 1) * L], u32)

    def halves(w):
        return (pltpu.bitcast(w << 16, f32), pltpu.bitcast(w & jnp.uint32(0xFFFF0000), f32))

    def gate(b, r0, n, l):
        base = pl.multiple_of(b * (T // 2), 8) + (l * (S + 16) + 16 + r0) // 2
        e0, a0 = halves(k_s[pl.ds(base, n // 2), :])
        e1, a1 = halves(k_s[pl.ds(base - 1, n // 2), :])
        _, a2 = halves(k_s[pl.ds(base - 2, n // 2), :])
        t0, t1, t2, t3 = (skt[t:t + 1, l * L:(l + 1) * L] for t in range(4))
        ve, va = halves(v_s[pk(b, r0, n), lanes(l)])
        ke = (e0 * t0 + a1 * t1 + e1 * t2 + a2 * t3) * ve
        ka = (a0 * t0 + e0 * t1 + a1 * t2 + e1 * t3) * va
        kv = jnp.concatenate([x[j:j + 8] for j in range(0, n // 2, 8) for x in (ke, ka)], 0)
        kv_s[l][pk(b, r0, n), :] = pltpu.bitcast(kv.astype(bf16), u32)

    q_cp(0).wait()
    layernorm(0, 0, 0, T)
    for l in range(NL):
        w_cp(w1_hbm, w1_s, l, 0).wait()

    def phase_a(i, _):
        nxt = jnp.minimum(i + 1, NA - 1)

        @pl.when(i + 1 < NA)
        def _():
            start_kvh(i + 1)
            q_cp(i + 1).wait()

        @pl.when(i + 2 < NA)
        def _():
            q_cp(i + 2).start()

        @pl.when(i == 2)
        def _():
            for l in range(NL):
                w_cp(w2_hbm, w2_s, l, 1).start()

        for l in range(NL):
            k_cp(i, l).wait()
        v_cp(i).wait()
        h_cp(i).wait()

        def mlp1(u, n):
            b = i * UA + u
            n0, n1 = n * L, min(F, (n + 1) * L)
            xn = jnp.concatenate([ld(xn_s[u % 2], b, l * S, T) for l in range(NL)], 1)
            w = jnp.concatenate([ld(w1_s, 0, l * F + n0, n1 - n0) for l in range(NL)], 1)
            z = jax.lax.dot_general(xn, w, _NT, preferred_element_type=f32)
            hook = z
            z = z + b1[:, n0:n1]
            t = jnp.tanh(z * (c1 + c2 * (z * z)))
            hz = 0.5 * z
            act_s[pk(b, n * S, T), 0:n1 - n0] = pltpu.bitcast((hz + hz * t).astype(bf16), u32)
            return hook

        def xdft(b, l):
            xf = jnp.dot(f_ref[2 * T:, :], ld(kv_s[l], b, 0, T), preferred_element_type=f32)
            xr, xi = xf[:T], xf[T:]
            xc_s[0, b, :, lanes(l)] = xr + xi
            xc_s[1, b, :, lanes(l)] = xr
            xc_s[2, b, :, lanes(l)] = xi

        def hdft(u, l):
            b = i * UA + u
            hf = jax.lax.dot_general(f_ref[:2 * T, :], h_s[i, lanes(l), u * T:(u + 1) * T], _NT,
                                     preferred_element_type=f32)
            hr, hi = hf[:T], hf[T:]
            pr, pi = hp_s[:T, lanes(l)], hp_s[T:, lanes(l)]
            H = T // 2
            gr = jnp.concatenate([hr[:H] - pi[:H], hr[H:] + pi[H:]], 0)
            gi = jnp.concatenate([hi[:H] + pr[:H], hi[H:] - pr[H:]], 0)
            if u == 0:
                gr = gr + jnp.where(i == 0, dd[:, l * L:(l + 1) * L], 0.0)
            hp_s[:, lanes(l)] = hf
            gc_s[0, b, :, lanes(l)] = gr
            gc_s[1, b, :, lanes(l)] = gi - gr
            gc_s[2, b, :, lanes(l)] = gr + gi

        nt = UA * NF
        sched = {j: [] for j in range(nt)}
        g_jobs = [(u, l, r) for u in range(UA) for l in range(NL) for r in range(0, T, GR)]
        for j, job in enumerate(g_jobs):
            pos = (G0 + (G1 - G0) * j / len(g_jobs)) * nt
            sched[int(pos)].append((pos % 1, "g", job))
            if job[2] == 0:
                sched[int(pos - HL)].append((-1, "h", job[:2]))
            if job[2] + GR == T:
                sched[int(pos + XL)].append((-1, "x", job[:2]))
        for u in range(UA):
            for j, r in enumerate(range(0, T, LR)):
                pos = (u + L0 + (L1 - L0) * j * LR / T) * NF
                sched[int(pos)].append((pos % 1, "ln", (u, r)))
        for j in range(nt):
            for _, kind, job in sorted(sched[j]):
                if kind == "h":
                    hdft(*job)
                elif kind == "x":
                    xdft(i * UA + job[0], job[1])
            z = mlp1(j // NF, j % NF)
            for frac, kind, job in sorted(sched[j]):
                r = int(max(frac, 0) * T) // 16 * 16
                hook = z[r:r + 16, 0:64].astype(bf16)
                if kind == "ln":
                    q_s[S:S + 16, 0:64] = hook
                    u = job[0] + 1
                    b = i * UA + u if u < UA else nxt * UA
                    layernorm(b, u % 2, job[1], LR)
                elif kind == "g":
                    k_s[pk(0, NL * (S + 16), 16), 0:64] = pltpu.bitcast(hook, u32)
                    gate(i * UA + job[0], job[2], GR, job[1])
        return 0

    jax.lax.fori_loop(0, NA, phase_a, 0)
    for l in range(NL):
        w_cp(w2_hbm, w2_s, l, 1).wait()

    def conv_piece(c, rows, ln, o0, o1):
        acc = {}
        for j in range(o1):
            b = xc_s[c, j, rows, ln]
            for o in range(max(o0, j), o1):
                p = gc_s[c, o - j, rows, ln] * b
                acc[o] = p if j == 0 else acc[o] + p
        for o in range(o0, o1):
            xc_s[c, o, rows, ln] = acc[o]

    pieces = [(u, c, l, o0, o1) for u in range(UB) for l in range(NL) for c in range(3)
              for (o0, o1) in ((13, 16), (9, 13), (0, 9))]
    chunks = [(u, l, k0, min(k0 + 4, NF)) for u in range(UB) for l in range(NL) for k0 in range(0, NF, 4)]

    def phase_b(i, _):
        total = UB * NL * NF
        t0 = 0
        nxt = 0
        acc = None
        for (u, l, k0, k1) in chunks:
            r0, r1 = k0 * L, min(F, k1 * L)
            b = i * UB + u
            lhs = jnp.concatenate([ld(act_s, b, n * S, T)[:, 0:min(F, (n + 1) * L) - n * L]
                                   for n in range(k0, k1)], 1)
            part = jnp.dot(lhs, ld(w2_s, 0, l * F + r0, r1 - r0), preferred_element_type=f32)
            t1 = t0 + (k1 - k0)
            while nxt < len(pieces) and nxt * total < t1 * len(pieces):
                pos = nxt * total / len(pieces)
                r = max(0, int((pos - t0) / (t1 - t0) * T)) // 8 * 8
                xc_s[3, 0, 0:8, 0:L] = part[r:r + 8]
                pu, c, pl_, o0, o1 = pieces[nxt]
                conv_piece(c, pl.ds(pl.multiple_of((i * UB + pu) * 8, 8), 8), lanes(pl_), o0, o1)
                nxt += 1
            t0 = t1
            acc = part + (b2[:, l * L:(l + 1) * L] if k0 == 0 else acc)
            if k1 == NF:
                mlp_s[rows_of(b * T, T), lanes(l)] = acc
        return 0

    jax.lax.fori_loop(0, NB // UB, phase_b, 0)

    def phase_c(i, _):
        for u in range(UC):
            b = i * UC + u
            k1 = xc_s[0, b]
            yc = jnp.concatenate([k1 - xc_s[2, b], k1 + xc_s[1, b]], 0).astype(bf16)
            y = jnp.dot(g_ref[...], yc, preferred_element_type=f32)
            xn = jnp.concatenate([ld(xn_s[u % 2], b, l * S, T) for l in range(NL)], 1)
            out = q_s[rows_of(b * T, T), :].astype(f32) + xn.astype(f32) * y + mlp_s[rows_of(b * T, T), :]
            o_s[rows_of(b * T, T), :] = out.astype(bf16)
            o_cp(b).start()
        return 0

    jax.lax.fori_loop(0, NB // UC, phase_c, 0)
    for i in range(NB):
        o_cp(i).wait()


@jax.jit
def pallas_parallel_sum__ssm_conv_h3__dense_activation_gelu__prompt_kernel(
    A_q: jax.Array,
    A_k: jax.Array,
    A_v: jax.Array,
    A_shift_k: jax.Array,
    A_ssm_k: jax.Array,
    A_ssm_D: jax.Array,
    B_x: jax.Array,
    B_w1: jax.Array,
    B_b1: jax.Array,
    B_w2: jax.Array,
    B_b2: jax.Array,
):
    del B_x
    _, S, D = A_q.shape
    F = B_w1.shape[1]
    NB = S // T
    NA = NB // UA
    NL = D // L
    NF = pl.cdiv(F, L)
    f32, bf16, u32 = jnp.float32, jnp.bfloat16, jnp.uint32
    hbm = pl.BlockSpec(memory_space=pltpu.HBM)
    vm = pl.BlockSpec(memory_space=pltpu.VMEM)
    return pl.pallas_call(
        _kernel,
        out_shape=jax.ShapeDtypeStruct(A_q.shape, A_q.dtype),
        in_specs=[hbm, hbm, hbm, vm, hbm, vm, hbm, vm, hbm, vm, vm, vm],
        out_specs=hbm,
        scratch_shapes=[
            pltpu.VMEM((S + 16, D), bf16),
            pltpu.VMEM((NL * (S + 16) // 2 + 8, L), u32),
            pltpu.VMEM((S // 2, D), u32),
            pltpu.VMEM((NA, D, UA * T), bf16),
            pltpu.VMEM((NL * F // 2, L), u32),
            pltpu.VMEM((NL * F // 2, L), u32),
            pltpu.VMEM((NL * S // 2, L), u32),
            pltpu.VMEM((NL * S // 2, L), u32),
            *[pltpu.VMEM((S // 2, L), u32)] * NL,
            pltpu.VMEM((NF * S // 2, L), u32),
            pltpu.VMEM((4, NB, T, D), f32),
            pltpu.VMEM((3, NB, T, D), f32),
            pltpu.VMEM((2 * T, D), f32),
            pltpu.VMEM((S, D), f32),
            pltpu.VMEM((S, D), bf16),
            pltpu.SemaphoreType.DMA((NA,)),
            pltpu.SemaphoreType.DMA((NA,)),
            pltpu.SemaphoreType.DMA((NA,)),
            pltpu.SemaphoreType.DMA((NA,)),
            pltpu.SemaphoreType.DMA((2,)),
            pltpu.SemaphoreType.DMA((NB,)),
        ],
        compiler_params=pltpu.CompilerParams(vmem_limit_bytes=110 * 1024 * 1024, disable_bounds_checks=True),
    )(A_q, A_k, A_v, A_shift_k.T, A_ssm_k, A_ssm_D, B_w1.T, B_b1, B_w2, B_b2,
      jnp.asarray(_FWD, dtype=bf16), jnp.asarray(_INV, dtype=bf16))
```

```python
import functools
import math

import jax
import jax.numpy as jnp
import numpy as np
import jax.experimental.pallas as pl
import jax.experimental.pallas.tpu as pltpu

T = 128
H = T // 2
L = 128
KC, NU, NC, FP = 4, 16, 4, 0.55
SPLIT = ((14, 16), (11, 14), (8, 11), (0, 8))
UA = 2
NP = 2
WC = 2
GR, LR = 64, 32
G0, G1, HL, XL = 0.1, 0.8, 1.0, 3.0
L0, L1 = 0.3, 0.8


def _dft_consts():
    k = np.concatenate([np.arange(0, T, 2), T - 1 - np.arange(0, T, 2)])
    n = np.arange(T)
    ang = np.pi * (2 * k[:, None] + 1) * n[None, :] / (2 * T)
    fwd = np.concatenate([np.cos(ang), -np.sin(ang)], 0)
    perm = (n // 16) * 16 + (n % 8) * 2 + (n // 8) % 2
    inv = np.concatenate([np.cos(ang[:H]).T, -np.sin(ang[:H]).T], 1) / T
    return np.concatenate([fwd, fwd[:, perm], inv[0::2], inv[1::2]], 0).astype(np.float32)


_DFT = _dft_consts()
_NT = (((1,), (1,)), ((), ()))


def _kernel(q_hbm, k_hbm, v_hbm, sk_hbm, h_hbm, d_hbm, w1_hbm, b1_hbm, w2_hbm, b2_hbm, f_hbm, o_hbm,
            q_s, k_s, v_s, h_s, w1_s, w2_s, xn0_s, xn1_s, xn2_s, kv0, kv1, kv2, kv3, kv4, act_s,
            xc_s, gc_s, kc_s, hp_s, mlp_s, y_s, o_s, sk_s, d_s, b1_s, b2_s, f_s, b1p_s, b2p_s,
            sq, sk, sv, sh, sw1, sw2, so, sc):
    _, S, D = q_hbm.shape
    F = w1_hbm.shape[0]
    NB = S // T
    NL = D // L
    NF = pl.cdiv(F, L)
    TA = UA * T
    NA = NB // UA
    NW = NF // WC
    f32, bf16, u32 = jnp.float32, jnp.bfloat16, jnp.uint32
    xn_s = (xn0_s, xn1_s, xn2_s)
    kv_s = (kv0, kv1, kv2, kv3, kv4)

    def rows_of(start, n):
        return pl.ds(pl.multiple_of(start, 16), n)

    def lanes(l):
        return pl.ds(l * L, L)

    def pk(b, off, n):
        return pl.ds(pl.multiple_of(b * H + off // 2, 8), n // 2)

    def as_bf16(w):
        return pltpu.bitcast(w, bf16)

    def halves(w):
        return (pltpu.bitcast(w << 16, f32), pltpu.bitcast(w & jnp.uint32(0xFFFF0000), f32))

    def q_cp(i):
        return pltpu.make_async_copy(q_hbm.at[0, rows_of(i * TA, TA)],
                                     q_s.bitcast(bf16).at[rows_of(i * TA, TA)], sq.at[i])

    def k_cp(i, l):
        return pltpu.make_async_copy(k_hbm.at[0, rows_of(i * TA, TA), lanes(l)],
                                     k_s.bitcast(bf16).at[rows_of(i * TA + l * (S + 16) + 16, TA)], sk.at[i])

    def v_cp(i):
        return pltpu.make_async_copy(v_hbm.at[0, rows_of(i * TA, TA)],
                                     v_s.bitcast(bf16).at[rows_of(i * TA, TA)], sv.at[i])

    def h_cp(i):
        return pltpu.make_async_copy(h_hbm.at[:, pl.ds(pl.multiple_of(i * TA, TA), TA)],
                                     h_s.bitcast(bf16).at[rows_of(i * D, D)], sh.at[i])

    def w1_cp(c, n):
        return pltpu.make_async_copy(w1_hbm.at[rows_of(c * WC * L, n)],
                                     w1_s.bitcast(bf16).at[rows_of(c * WC * L, n)], sw1.at[c])

    w2_cp = pltpu.make_async_copy(w2_hbm, w2_s.bitcast(bf16).at[pl.ds(0, F)], sw2.at[0])
    small = [pltpu.make_async_copy(a, b, sc.at[j]) for j, (a, b) in enumerate(
        ((b1_hbm, b1_s), (sk_hbm, sk_s), (d_hbm, d_s), (b2_hbm, b2_s), (f_hbm, f_s.bitcast(bf16))))]
    last_w1 = F - (NW - 1) * WC * L

    def start_kvh(i):
        for l in range(NL):
            k_cp(i, l).start()
        v_cp(i).start()
        h_cp(i).start()

    def wait_kvh(i):
        for l in range(NL):
            k_cp(i, l).wait()
        v_cp(i).wait()
        h_cp(i).wait()

    q_cp(0).start()
    small[0].start()
    w1_cp(0, WC * L).start()
    for i in range(1, NP):
        q_cp(i).start()
    for c in range(1, NW):
        w1_cp(c, WC * L if c < NW - 1 else last_w1).start()
    for cp in small[1:]:
        cp.start()
    q_cp(NP).start()
    q_cp(NP + 1).start()
    start_kvh(0)
    q_cp(NP + 2).start()
    start_kvh(1)

    for l in range(NL):
        k_s[pk(0, l * (S + 16), 16), :] = jnp.zeros((8, L), u32)
    hp_s[...] = jnp.zeros(hp_s.shape, f32)
    mlp_s[:, lanes(0)] = jnp.zeros((S, L), f32)
    kc_s[:, :, :, lanes(0)] = jnp.zeros((3, NB, T, L), f32)
    pad = NF * L - F
    w1_s[pk(0, F, pad), :] = jnp.zeros((pad // 2, D), u32)
    w2_s[pk(0, F, pad), :] = jnp.zeros((pad // 2, D), u32)
    c1 = math.sqrt(2.0 / math.pi)
    c2 = c1 * 0.044715

    def layernorm(b, par, r0, n):
        for j, x in enumerate(halves(q_s[pk(b, r0, n), :])):
            m = jnp.mean(x, axis=-1, keepdims=True)
            xc = x - m
            var = jnp.mean(xc * xc, axis=-1, keepdims=True)
            xn = (xc * jax.lax.rsqrt(var + 1e-5)).astype(bf16)
            for dst in (par, 2):
                xn_s[dst][pk(b, j * H + r0 // 2, n // 2), :] = pltpu.bitcast(xn, u32)

    def mlp1(b, par, n):
        z = jax.lax.dot_general(as_bf16(xn_s[par][pk(b, 0, T), :]), as_bf16(w1_s[pk(n, 0, L), :]), _NT,
                                preferred_element_type=f32)
        a = z + b1p_s[n, 0:1, :]
        t = jnp.tanh(a * (c1 + c2 * (a * a)))
        act_s[n, pk(b, 0, T), :] = pltpu.bitcast((a + a * t).astype(bf16), u32)
        return z

    def gate(b, r0, n, l):
        base = pl.multiple_of(b * H, 8) + (l * (S + 16) + 16 + r0) // 2
        e0, a0 = halves(k_s[pl.ds(base, n // 2), :])
        e1, a1 = halves(k_s[pl.ds(base - 1, n // 2), :])
        _, a2 = halves(k_s[pl.ds(base - 2, n // 2), :])
        t0, t1, t2, t3 = (sk_s[t:t + 1, lanes(l)].astype(f32) for t in range(4))
        ve, va = halves(v_s[pk(b, r0, n), lanes(l)])
        ke = (e0 * t0 + a1 * t1 + e1 * t2 + a2 * t3) * ve
        ka = (a0 * t0 + e0 * t1 + a1 * t2 + e1 * t3) * va
        kv = jnp.concatenate([x[j:j + 8] for j in range(0, n // 2, 8) for x in (ke, ka)], 0)
        kv_s[l][pk(b, r0, n), :] = pltpu.bitcast(kv.astype(bf16), u32)

    def xdft(b, l):
        xf = jnp.dot(as_bf16(f_s[T:2 * T, :]), as_bf16(kv_s[l][pk(b, 0, T), :]), preferred_element_type=f32)
        xr, xi = xf[:T], xf[T:]
        xc_s[0, b, :, lanes(l)] = xr + xi
        xc_s[1, b, :, lanes(l)] = xr
        xc_s[2, b, :, lanes(l)] = xi

    def hdft(i, u, l):
        b = i * UA + u
        hb = as_bf16(h_s[pl.ds(pl.multiple_of(i * (D // 2), 8) + l * H, H), u * T:(u + 1) * T])
        hf = jax.lax.dot_general(as_bf16(f_s[0:T, :]), hb, _NT, preferred_element_type=f32)
        hr, hi = hf[:T], hf[T:]
        pr, pi = hp_s[:T, lanes(l)], hp_s[T:, lanes(l)]
        gr = jnp.concatenate([hr[:H] - pi[:H], hr[H:] + pi[H:]], 0)
        gi = jnp.concatenate([hi[:H] + pr[:H], hi[H:] - pr[H:]], 0)
        if u == 0:
            dd = d_s[...].astype(f32).reshape(1, D)
            gr = gr + jnp.where(i == 0, dd[:, l * L:(l + 1) * L], 0.0)
        hp_s[:, lanes(l)] = hf
        gc_s[0, b, :, lanes(l)] = gr
        gc_s[1, b, :, lanes(l)] = gi - gr
        gc_s[2, b, :, lanes(l)] = gr + gi

    small[0].wait()
    b1 = b1_s[...].astype(f32).reshape(1, F)
    b1p_s[NF - 1] = jnp.zeros((8, L), f32)
    for n in range(NF):
        w = min(L, F - n * L)
        b1p_s[n, 0:1, 0:w] = b1[:, n * L:n * L + w]
    for i in range(NP):
        q_cp(i).wait()
        for u in range(UA):
            layernorm(i * UA + u, u % 2, 0, T)

    def phase_p(c, _):
        @pl.when(c < NW - 1)
        def _():
            w1_cp(c, WC * L).wait()

        @pl.when(c == NW - 1)
        def _():
            w1_cp(NW - 1, last_w1).wait()

        for b in range(NP * UA):
            for n in range(WC):
                mlp1(b, b % 2, c * WC + n)
        return 0

    jax.lax.fori_loop(0, NW, phase_p, 0)
    for cp in small[1:]:
        cp.wait()
    b2 = b2_s[...].astype(f32).reshape(1, D)
    for l in range(NL):
        b2p_s[l, 0:1, :] = b2[:, l * L:(l + 1) * L]
    q_cp(NP).wait()
    layernorm(NP * UA, 0, 0, T)

    def phase_a(i, _):
        im = i + NP
        nxt = jnp.minimum(im + 1, NA - 1)

        @pl.when(i == 1)
        def _():
            for j in range(2, NA):
                if j + NP + 1 < NA:
                    q_cp(j + NP + 1).start()
                start_kvh(j)
            w2_cp.start()

        @pl.when(im + 1 < NA)
        def _():
            q_cp(im + 1).wait()

        wait_kvh(i)
        nt = UA * NF
        sched = {j: [] for j in range(nt)}
        g_jobs = [(u, l, r) for u in range(UA) for l in range(NL) for r in range(0, T, GR)]
        for j, job in enumerate(g_jobs):
            pos = (G0 + (G1 - G0) * j / len(g_jobs)) * nt
            sched[int(pos)].append((pos % 1, "g", job))
            if job[2] == 0:
                sched[int(pos - HL)].append((-1, "h", job[:2]))
            if job[2] + GR == T:
                sched[int(pos + XL)].append((-1, "x", job[:2]))
        for u in range(UA):
            for j, r in enumerate(range(0, T, LR)):
                pos = (u + L0 + (L1 - L0) * j * LR / T) * NF
                sched[int(pos)].append((pos % 1, "ln", (u, r)))
        for j in range(nt):
            for _, kind, job in sorted(sched[j]):
                if kind == "h":
                    hdft(i, *job)
                elif kind == "x":
                    xdft(i * UA + job[0], job[1])
            z = mlp1(im * UA + j // NF, (j // NF) % 2, j % NF)
            for frac, kind, job in sorted(sched[j]):
                r = int(max(frac, 0) * T) // 8 * 8
                hook = pltpu.bitcast(z[r:r + 8], u32)
                if kind == "ln":
                    q_s[S // 2:S // 2 + 8, 0:L] = hook
                    u = job[0] + 1
                    layernorm(im * UA + u if u < UA else nxt * UA, u % 2, job[1], LR)
                elif kind == "g":
                    k_s[pk(0, NL * (S + 16), 16), :] = hook
                    gate(i * UA + job[0], job[2], GR, job[1])
        return 0

    jax.lax.fori_loop(0, NA - NP, phase_a, 0)

    def phase_e(i, _):
        wait_kvh(i)
        for u in range(UA):
            for l in range(NL):
                hdft(i, u, l)
                gate(i * UA + u, 0, T, l)
        for u in range(UA):
            for l in range(NL):
                xdft(i * UA + u, l)
        return 0

    jax.lax.fori_loop(NA - NP, NA, phase_e, 0)
    w2_cp.wait()

    def dyn_lanes(l):
        return pl.ds(pl.multiple_of(l * L, L), L)

    def mlp2(b, l, jobs):
        ln = dyn_lanes(l)
        acc = None
        done = 0
        for k0 in range(0, NF, KC):
            k1 = min(k0 + KC, NF)
            lhs = jnp.concatenate([as_bf16(act_s[n, pk(b, 0, T), :]) for n in range(k0, k1)], 1)
            part = jnp.dot(lhs, as_bf16(w2_s[pk(k0, 0, (k1 - k0) * L), ln]), preferred_element_type=f32)
            while done < len(jobs) and jobs[done][0] * NF < k1:
                r = max(0, int((jobs[done][0] * NF - k0) / (k1 - k0) * T)) // 8 * 8
                xc_s[3, 0, 0:8, 0:L] = part[r:r + 8]
                jobs[done][1]()
                done += 1
            acc = part if k0 == 0 else acc + part
        x = jnp.concatenate(halves(q_s[pk(b, 0, T), ln]), 0)
        mlp_s[rows_of(b * T, T), ln] = 0.5 * acc + (x + b2p_s[l, 0:1, :])

    def conv_piece(c, rows, ln, o0, o1):
        acc = {}
        for j in range(o1):
            b = xc_s[c, j, rows, ln]
            for o in range(max(o0, j), o1):
                p = gc_s[c, o - j, rows, ln] * b
                acc[o] = p if j == 0 else acc[o] + p
        for o in range(o0, o1):
            kc_s[c, o, rows, ln] = acc[o]

    def fold(b, ln, slot):
        k1 = kc_s[0, b, :, ln]
        yr, yi = k1 - kc_s[2, b, :, ln], k1 + kc_s[1, b, :, ln]
        y = jnp.concatenate([yr[:H] + yr[H:], yi[:H] - yi[H:], yr[:H] - yr[H:], yi[:H] + yi[H:]], 0)
        y_s[slot] = pltpu.bitcast(y.astype(bf16), u32)

    def finish(b, ln, slot):
        y = jnp.concatenate([
            jnp.dot(as_bf16(f_s[2 * T + j * H // 2:2 * T + (j + 1) * H // 2, :]),
                    as_bf16(y_s[slot, j * H:(j + 1) * H, :]), preferred_element_type=f32)
            for j in range(2)], 0)
        out = as_bf16(xn_s[2][pk(b, 0, T), ln]).astype(f32) * y + mlp_s[rows_of(b * T, T), ln]
        o_s[pk(b, 0, T), ln] = pltpu.pack_elementwise([out[:H], out[H:]], packed_dtype=bf16)

    NH = NB // NU

    def o_cp(i, l, b, n):
        src = (rows_of(b * T, n * T), dyn_lanes(l))
        return pltpu.make_async_copy(o_s.bitcast(bf16).at[src], o_hbm.at[(0,) + src], so.at[i])

    def phase_b(i, _):
        l, h = i // NH, i % NH
        lp = dyn_lanes(jnp.maximum(l - 1, 0))
        for j in range(NU):
            b = h * NU + j
            rows = pl.ds(pl.multiple_of(b * 8, 8), 8)
            jobs = [functools.partial(fold, b, lp, j)]
            jobs += [functools.partial(conv_piece, c, rows, dyn_lanes(l), o0, o1)
                     for c in range(3) for (o0, o1) in SPLIT]
            jobs = [(p / len(jobs), job) for p, job in enumerate(jobs)]
            jobs.append((FP, functools.partial(finish, b, lp, j)))
            mlp2(b, l, sorted(jobs, key=lambda x: x[0]))

        @pl.when(l > 0)
        def _():
            o_cp(i, l - 1, h * NU, NU).start()
        return 0

    jax.lax.fori_loop(0, NL * NH, phase_b, 0)

    def phase_c(i, _):
        for j in range(NC):
            fold(i * NC + j, lanes(NL - 1), j)
        for j in range(NC):
            finish(i * NC + j, lanes(NL - 1), j)
        o_cp(NL * NH + i, NL - 1, i * NC, NC).start()
        return 0

    jax.lax.fori_loop(0, NB // NC, phase_c, 0)
    for i in range(NH, NL * NH):
        o_cp(i, i // NH - 1, i % NH * NU, NU).wait()
    for i in range(NB // NC):
        o_cp(NL * NH + i, NL - 1, i * NC, NC).wait()


@jax.jit
def pallas_parallel_sum__ssm_conv_h3__dense_activation_gelu__prompt_kernel(
    A_q: jax.Array,
    A_k: jax.Array,
    A_v: jax.Array,
    A_shift_k: jax.Array,
    A_ssm_k: jax.Array,
    A_ssm_D: jax.Array,
    B_x: jax.Array,
    B_w1: jax.Array,
    B_b1: jax.Array,
    B_w2: jax.Array,
    B_b2: jax.Array,
):
    del B_x
    _, S, D = A_q.shape
    F = B_w1.shape[1]
    NB = S // T
    NA = NB // UA
    NL = D // L
    NF = pl.cdiv(F, L)
    f32, bf16, u32 = jnp.float32, jnp.bfloat16, jnp.uint32
    hbm = pl.BlockSpec(memory_space=pltpu.HBM)
    dma = pltpu.SemaphoreType.DMA
    return pl.pallas_call(
        _kernel,
        out_shape=jax.ShapeDtypeStruct(A_q.shape, A_q.dtype),
        in_specs=[hbm] * 11,
        out_specs=hbm,
        scratch_shapes=[
            pltpu.VMEM((S // 2 + 8, D), u32),
            pltpu.VMEM((NL * (S + 16) // 2 + 8, L), u32),
            pltpu.VMEM((S // 2, D), u32),
            pltpu.VMEM((NA * D // 2, UA * T), u32),
            pltpu.VMEM((NF * H, D), u32),
            pltpu.VMEM((NF * H, D), u32),
            pltpu.VMEM((S // 2, D), u32),
            pltpu.VMEM((S // 2, D), u32),
            pltpu.VMEM((S // 2, D), u32),
            *[pltpu.VMEM((S // 2, L), u32)] * NL,
            pltpu.VMEM((NF, S // 2, L), u32),
            pltpu.VMEM((4, NB, T, D), f32),
            pltpu.VMEM((3, NB, T, D), f32),
            pltpu.VMEM((3, NB, T, D), f32),
            pltpu.VMEM((2 * T, D), f32),
            pltpu.VMEM((S, D), f32),
            pltpu.VMEM((NU, T, L), u32),
            pltpu.VMEM((S // 2, D), u32),
            pltpu.VMEM(A_shift_k.shape[::-1], bf16),
            pltpu.VMEM((D,), bf16),
            pltpu.VMEM((F,), bf16),
            pltpu.VMEM((D,), bf16),
            pltpu.VMEM((_DFT.shape[0] // 2, T), u32),
            pltpu.VMEM((NF, 8, L), f32),
            pltpu.VMEM((NL, 8, L), f32),
            dma((NA,)), dma((NA,)), dma((NA,)), dma((NA,)), dma((NF // WC,)), dma((1,)), dma((NL * NB // NU + NB // NC,)), dma((5,)),
        ],
        compiler_params=pltpu.CompilerParams(vmem_limit_bytes=110 * 1024 * 1024, disable_bounds_checks=True),
    )(A_q, A_k, A_v, A_shift_k.T, A_ssm_k, A_ssm_D, B_w1.T, B_b1, B_w2, B_b2, jnp.asarray(_DFT, dtype=bf16))
```

```python
import functools
import math

import jax
import jax.numpy as jnp
import numpy as np
import jax.experimental.pallas as pl
import jax.experimental.pallas.tpu as pltpu

T = 128
H = T // 2
L = 128
KC, MU, FP = (0, 6, 10, 14), 15, 0.55
LAST = ((3, 0, 11), (2, 11, 16))
J0, J1 = 0.0, 1.0
SPLIT = ((14, 16), (11, 14), (8, 11), (0, 8))
UA, CQ = 2, 3
FL = {}
PX, PG, PK = 8, 8, 8
NP = 2
WC = 2
GR, LR = 64, 32
G0, G1, HL, XL = 0.1, 0.8, 1.0, 3.0
L0, L1 = 0.3, 0.8


def _dft_consts():
    k = np.concatenate([np.arange(0, T, 2), T - 1 - np.arange(0, T, 2)])
    n = np.arange(T)
    ang = np.pi * (2 * k[:, None] + 1) * n[None, :] / (2 * T)
    fwd = np.concatenate([np.cos(ang), -np.sin(ang)], 0)
    perm = (n // 16) * 16 + (n % 8) * 2 + (n // 8) % 2
    inv = np.concatenate([np.cos(ang[:H]).T, -np.sin(ang[:H]).T], 1) / T
    r = np.arange(2 * T)
    fwd = fwd[(r // 16) * 8 + r % 8 + (r // 8) % 2 * T]
    return np.concatenate([fwd, fwd[:, perm], inv[0::2], inv[1::2]], 0).astype(np.float32)


_DFT = _dft_consts()
_NT = (((1,), (1,)), ((), ()))


def _kernel(q_hbm, k_hbm, v_hbm, sk_hbm, h_hbm, d_hbm, w1_hbm, b1_hbm, w2_hbm, b2_hbm, f_hbm, o_hbm,
            q_s, k_s, v_s, h_s, w1_s, w2_s, xn0_s, xn1_s, xn2_s, kv0, kv1, kv2, kv3, kv4, act_s,
            xc_s, gc_s, kc_s, hp_s, mlp_s, y_s, o_s, sk_s, d_s, b1_s, b2_s, f_s, b1p_s, b2p_s, fill_s,
            sq, sk, sv, sh, sw1, sw2, so, sc):
    _, S, D = q_hbm.shape
    F = w1_hbm.shape[0]
    NB = S // T
    NL = D // L
    NF = pl.cdiv(F, L)
    TA = UA * T
    NA = NB // UA
    NW = NF // WC
    f32, bf16, u32 = jnp.float32, jnp.bfloat16, jnp.uint32
    xn_s = (xn0_s, xn1_s, xn2_s)
    kv_s = (kv0, kv1, kv2, kv3, kv4)

    def rows_of(start, n):
        return pl.ds(pl.multiple_of(start, 16), n)

    def lanes(l):
        return pl.ds(l * L, L)

    def pk(b, off, n):
        return pl.ds(pl.multiple_of(b * H + off // 2, 8), n // 2)

    def as_bf16(w):
        return pltpu.bitcast(w, bf16)

    def halves(w):
        return (pltpu.bitcast(w << 16, f32), pltpu.bitcast(w & jnp.uint32(0xFFFF0000), f32))

    def q_cp(i):
        return pltpu.make_async_copy(q_hbm.at[0, rows_of(i * TA, TA)],
                                     q_s.bitcast(bf16).at[rows_of(i * TA, TA)], sq.at[i])

    def k_cp(i, l):
        return pltpu.make_async_copy(k_hbm.at[0, rows_of(i * TA, TA), lanes(l)],
                                     k_s.bitcast(bf16).at[rows_of(i * TA + l * (S + 16) + 16, TA)], sk.at[i])

    def v_cp(i):
        return pltpu.make_async_copy(v_hbm.at[0, rows_of(i * TA, TA)],
                                     v_s.bitcast(bf16).at[rows_of(i * TA, TA)], sv.at[i])

    def h_cp(i):
        return pltpu.make_async_copy(h_hbm.at[:, pl.ds(pl.multiple_of(i * TA, TA), TA)],
                                     h_s.bitcast(bf16).at[rows_of(i * D, D)], sh.at[i])

    def w1_cp(c, n):
        return pltpu.make_async_copy(w1_hbm.at[rows_of(c * WC * L, n)],
                                     w1_s.bitcast(bf16).at[rows_of(c * WC * L, n)], sw1.at[c])

    w2_cp = pltpu.make_async_copy(w2_hbm, w2_s.bitcast(bf16).at[pl.ds(0, F)], sw2.at[0])
    small = [pltpu.make_async_copy(a, b, sc.at[j]) for j, (a, b) in enumerate(
        ((b1_hbm, b1_s), (sk_hbm, sk_s), (d_hbm, d_s), (b2_hbm, b2_s), (f_hbm, f_s.bitcast(bf16))))]
    last_w1 = F - (NW - 1) * WC * L

    def start_kvh(i):
        for l in range(NL):
            k_cp(i, l).start()
        v_cp(i).start()
        h_cp(i).start()

    def wait_kvh(i):
        for l in range(NL):
            k_cp(i, l).wait()
        v_cp(i).wait()
        h_cp(i).wait()

    q_cp(0).start()
    small[0].start()
    w1_cp(0, WC * L).start()
    for i in range(1, NP):
        q_cp(i).start()
    for c in range(1, NW):
        w1_cp(c, WC * L if c < NW - 1 else last_w1).start()
        if c == CQ - 1:
            q_cp(NP).start()
    pltpu.make_async_copy(w1_hbm.at[pl.ds(0, WC * L - last_w1)], fill_s.bitcast(bf16), sw1.at[NW - 1]).start()
    for cp in small[1:]:
        cp.start()
    q_cp(NP + 1).start()
    start_kvh(0)
    q_cp(NP + 2).start()
    start_kvh(1)

    for l in range(NL):
        k_s[pk(0, l * (S + 16), 16), :] = jnp.zeros((8, L), u32)
    hp_s[...] = jnp.zeros(hp_s.shape, f32)
    mlp_s[:, lanes(0)] = jnp.zeros((S, L), f32)
    kc_s[:, :, :T, lanes(0)] = jnp.zeros((3, NB, T, L), f32)
    pad = NF * L - F
    w1_s[pk(0, F, pad), :] = jnp.zeros((pad // 2, D), u32)
    w2_s[pk(0, F, pad), :] = jnp.zeros((pad // 2, D), u32)
    c1 = math.sqrt(2.0 / math.pi)
    c2 = c1 * 0.044715

    def layernorm(b, par, r0, n):
        for j, x in enumerate(halves(q_s[pk(b, r0, n), :])):
            m = jnp.mean(x, axis=-1, keepdims=True)
            xc = x - m
            var = jnp.mean(xc * xc, axis=-1, keepdims=True)
            xn = (xc * jax.lax.rsqrt(var + 1e-5)).astype(bf16)
            for dst in (par, 2):
                xn_s[dst][pk(b, j * H + r0 // 2, n // 2), :] = pltpu.bitcast(xn, u32)

    def mlp1(b, par, n):
        z = jax.lax.dot_general(as_bf16(xn_s[par][pk(b, 0, T), :]), as_bf16(w1_s[pk(n, 0, L), :]), _NT,
                                preferred_element_type=f32)
        a = z + b1p_s[n, 0:1, :]
        t = jnp.tanh(a * (c1 + c2 * (a * a)))
        act_s[n, pk(b, 0, T), :] = pltpu.bitcast((a + a * t).astype(bf16), u32)
        return z

    def gate(b, r0, n, l):
        base = pl.multiple_of(b * H, 8) + (l * (S + 16) + 16 + r0) // 2
        e0, a0 = halves(k_s[pl.ds(base, n // 2), :])
        e1, a1 = halves(k_s[pl.ds(base - 1, n // 2), :])
        _, a2 = halves(k_s[pl.ds(base - 2, n // 2), :])
        t0, t1, t2, t3 = (sk_s[t:t + 1, lanes(l)].astype(f32) for t in range(4))
        ve, va = halves(v_s[pk(b, r0, n), lanes(l)])
        ke = (e0 * t0 + a1 * t1 + e1 * t2 + a2 * t3) * ve
        ka = (a0 * t0 + e0 * t1 + a1 * t2 + e1 * t3) * va
        kv = jnp.concatenate([x[j:j + 8] for j in range(0, n // 2, 8) for x in (ke, ka)], 0)
        kv_s[l][pk(b, r0, n), :] = pltpu.bitcast(kv.astype(bf16), u32)

    def re_im(f):
        return tuple(jnp.concatenate([f[r + o:r + o + 8] for r in range(0, 2 * T, 16)], 0) for o in (0, 8))

    def xdft(b, l):
        xr, xi = re_im(jnp.dot(as_bf16(f_s[T:2 * T, :]), as_bf16(kv_s[l][pk(b, 0, T), :]),
                               preferred_element_type=f32))
        xc_s[0, b, :T, lanes(l)] = xr + xi
        xc_s[1, b, :T, lanes(l)] = xr
        xc_s[2, b, :T, lanes(l)] = xi

    def hpair(i, l, first=True, keep=True):
        prev = hp_s[:, lanes(l)]
        for u in range(UA):
            hb = as_bf16(h_s[pl.ds(pl.multiple_of(i * (D // 2), 8) + l * H, H), u * T:(u + 1) * T])
            hf = jax.lax.dot_general(as_bf16(f_s[0:T, :]), hb, _NT, preferred_element_type=f32)
            hr, hi = re_im(hf)
            pr, pi = re_im(prev)
            gr = jnp.concatenate([hr[:H] - pi[:H], hr[H:] + pi[H:]], 0)
            gi = jnp.concatenate([hi[:H] + pr[:H], hi[H:] - pr[H:]], 0)
            if u == 0 and first:
                dd = d_s[...].astype(f32).reshape(1, D)
                gr = gr + jnp.where(i == 0, dd[:, l * L:(l + 1) * L], 0.0)
            b = i * UA + u
            gc_s[0, b, :T, lanes(l)] = gr
            gc_s[1, b, :T, lanes(l)] = gi - gr
            gc_s[2, b, :T, lanes(l)] = gr + gi
            prev = hf
        if keep:
            hp_s[:, lanes(l)] = prev

    small[0].wait()
    b1 = b1_s[...].astype(f32).reshape(1, F)
    b1p_s[NF - 1] = jnp.zeros((8, L), f32)
    for n in range(NF):
        w = min(L, F - n * L)
        b1p_s[n, 0:1, 0:w] = b1[:, n * L:n * L + w]
    for i in range(NP):
        q_cp(i).wait()
        for u in range(UA):
            layernorm(i * UA + u, u % 2, 0, T)

    def phase_p(c, _):
        w1_cp(c, WC * L).wait()

        @pl.when(c == CQ)
        def _():
            q_cp(NP).wait()

        for b in (0, 2, 1, 3):
            for n in range(WC):
                z = mlp1(b, b % 2, c * WC + n)
                if b == 1:
                    for r in range(0, H, LR):
                        q_s[S // 2:S // 2 + 8, 0:L] = pltpu.bitcast(z[2 * r:2 * r + 8], u32)
                        layernorm(jnp.where(c < CQ, 0, NP * UA), 0, n * H + r, LR)
        return 0

    jax.lax.fori_loop(0, NW, phase_p, 0)
    for cp in small[1:]:
        cp.wait()
    b2 = b2_s[...].astype(f32).reshape(1, D)
    for l in range(NL):
        b2p_s[l, 0:1, :] = b2[:, l * L:(l + 1) * L]

    def phase_a(i, _):
        im = i + NP
        nxt = jnp.minimum(im + 1, NA - 1)

        @pl.when(i == 1)
        def _():
            for j in range(2, NA):
                if j + NP + 1 < NA:
                    q_cp(j + NP + 1).start()
                start_kvh(j)
            w2_cp.start()

        @pl.when(im + 1 < NA)
        def _():
            q_cp(im + 1).wait()

        wait_kvh(i)
        nt = UA * NF
        sched = {j: [] for j in range(nt)}
        g_jobs = [(u, l, r) for u in range(UA) for l in range(NL) for r in range(0, T, GR)]
        for j, job in enumerate(g_jobs):
            pos = (G0 + (G1 - G0) * j / len(g_jobs)) * nt
            sched[int(pos)].append((pos % 1, "g", job))
            if j % (len(g_jobs) // NL) == 0:
                sched[int(pos - HL)].append((-1, "h", j // (len(g_jobs) // NL)))
            if job[2] + GR == T:
                sched[int(pos + XL)].append((-1, "x", job[:2]))
        for u in range(UA):
            for j, r in enumerate(range(0, T, LR)):
                pos = (u + L0 + (L1 - L0) * j * LR / T) * NF
                sched[int(pos)].append((pos % 1, "ln", (u, r)))
        for j in range(nt):
            for _, kind, job in sorted(sched[j]):
                if kind == "h":
                    hpair(i, job)
                elif kind == "x":
                    xdft(i * UA + job[0], job[1])
            z = mlp1(im * UA + j // NF, (j // NF) % 2, j % NF)
            for frac, kind, job in sorted(sched[j]):
                r = int(max(frac, 0) * T) // 8 * 8
                hook = pltpu.bitcast(z[r:r + 8], u32)
                if kind == "ln":
                    q_s[S // 2:S // 2 + 8, 0:L] = hook
                    u = job[0] + 1
                    layernorm(im * UA + u if u < UA else nxt * UA, u % 2, job[1], LR)
                elif kind == "g":
                    k_s[pk(0, NL * (S + 16), 16), :] = hook
                    gate(i * UA + job[0], job[2], GR, job[1])
        return 0

    jax.lax.fori_loop(0, NA - NP, phase_a, 0)

    for i in range(NA - NP, NA):
        wait_kvh(i)
    for i in range(NA - NP, NA):
        for l in range(NL):
            hpair(i, l, first=False, keep=i + 1 < NA)
            for u in range(UA):
                gate(i * UA + u, 0, T, l)
            if i > NA - NP:
                for u in range(UA):
                    xdft((i - 1) * UA + u, l)
    for l in range(NL):
        for u in range(UA):
            xdft((NA - 1) * UA + u, l)
    w2_cp.wait()

    def dyn_lanes(l):
        return pl.ds(pl.multiple_of(l * L, L), L)

    def mlp2(b, l, jobs):
        ln = dyn_lanes(l)
        acc = None
        done = 0
        for k0, k1 in zip(KC, KC[1:]):
            lhs = jnp.concatenate([as_bf16(act_s[n, pk(b, 0, T), :]) for n in range(k0, k1)], 1)
            part = jnp.dot(lhs, as_bf16(w2_s[pk(k0, 0, (k1 - k0) * L), ln]), preferred_element_type=f32)
            while done < len(jobs) and jobs[done][0] * NF < k1:
                r = max(0, int((jobs[done][0] * NF - k0) / (k1 - k0) * T)) // 8 * 8
                xc_s[3, 0, 0:8, 0:L] = part[r:r + 8]
                jobs[done][1]()
                done += 1
            acc = part if k0 == 0 else acc + part
        x = jnp.concatenate(halves(q_s[pk(b, 0, T), ln]), 0)
        mlp_s[rows_of(b * T, T), ln] = 0.5 * acc + (x + b2p_s[l, 0:1, :])

    def conv_piece(c, rows, ln, o0, o1):
        acc = {}
        for j in range(o1):
            b = xc_s[c, j, rows, ln]
            for o in range(max(o0, j), o1):
                p = gc_s[c, o - j, rows, ln] * b
                acc[o] = p if j == 0 else acc[o] + p
        for o in range(o0, o1):
            kc_s[c, o, rows, ln] = acc[o]

    def fold(b, ln, slot):
        k1 = kc_s[0, b, :T, ln]
        yr, yi = k1 - kc_s[2, b, :T, ln], k1 + kc_s[1, b, :T, ln]
        y = jnp.concatenate([yr[:H] + yr[H:], yi[:H] - yi[H:], yr[:H] - yr[H:], yi[:H] + yi[H:]], 0)
        y_s[slot] = pltpu.bitcast(y.astype(bf16), u32)

    def finish(b, ln, slot):
        y = jnp.concatenate([
            jnp.dot(as_bf16(f_s[2 * T + j * H // 2:2 * T + (j + 1) * H // 2, :]),
                    as_bf16(y_s[slot, j * H:(j + 1) * H, :]), preferred_element_type=f32)
            for j in range(2)], 0)
        out = as_bf16(xn_s[2][pk(b, 0, T), ln]).astype(f32) * y + mlp_s[rows_of(b * T, T), ln]
        o_s[pk(b, 0, T), ln] = pltpu.pack_elementwise([out[:H], out[H:]], packed_dtype=bf16)


    def o_cp(i, l, b, n):
        src = (rows_of(b * T, n * T), dyn_lanes(l))
        return pltpu.make_async_copy(o_s.bitcast(bf16).at[src], o_hbm.at[(0,) + src], so.at[i])

    def run_units(first, count, jobs):
        for j in range(count):
            todo = sorted([(p * count - j, job) for p, job in jobs if j <= p * count < j + 1], key=lambda x: x[0])
            mlp2((first + j) % NB, (first + j) // NB, todo)

    def phase_b(l, _):
        lp = dyn_lanes(jnp.maximum(l - 1, 0))
        jobs = []
        for b in range(NB):
            jobs.append(functools.partial(fold, b, lp, b))
            jobs += [functools.partial(conv_piece, c, pl.ds(b * 8, 8), dyn_lanes(l), o0, o1)
                     for c in range(3) for (o0, o1) in SPLIT]
        jobs = [(J0 + (J1 - J0) * p / len(jobs), job) for p, job in enumerate(jobs)]
        jobs += [((min(b, MU - 1) + FP) / MU, functools.partial(finish, b, lp, b)) for b in range(NB)]
        run_units(l * MU, MU, jobs)

        @pl.when(l > 0)
        def _():
            o_cp(l, l - 1, 0, NB).start()
        return 0

    jax.lax.fori_loop(0, NL, phase_b, 0)

    first = NL * MU
    for i, (n, b0, b1) in enumerate(LAST):
        jobs = [(0.8 * (b - b0) / (b1 - b0), functools.partial(fold, b, lanes(NL - 1), b)) for b in range(b0, b1)]
        jobs += [(0.8 * (b + 1.5 - b0) / (b1 - b0), functools.partial(finish, b, lanes(NL - 1), b))
                 for b in range(b0, b1 - 1)]
        run_units(first, n, jobs)
        finish(b1 - 1, lanes(NL - 1), b1 - 1)
        o_cp(NL + i, NL - 1, b0, b1 - b0).start()
        first += n
    for l in range(1, NL):
        o_cp(l, l - 1, 0, NB).wait()
    for i, (n, b0, b1) in enumerate(LAST):
        o_cp(NL + i, NL - 1, b0, b1 - b0).wait()


@jax.jit
def pallas_parallel_sum__ssm_conv_h3__dense_activation_gelu__prompt_kernel(
    A_q: jax.Array,
    A_k: jax.Array,
    A_v: jax.Array,
    A_shift_k: jax.Array,
    A_ssm_k: jax.Array,
    A_ssm_D: jax.Array,
    B_x: jax.Array,
    B_w1: jax.Array,
    B_b1: jax.Array,
    B_w2: jax.Array,
    B_b2: jax.Array,
):
    del B_x
    _, S, D = A_q.shape
    F = B_w1.shape[1]
    NB = S // T
    NA = NB // UA
    NL = D // L
    NF = pl.cdiv(F, L)
    f32, bf16, u32 = jnp.float32, jnp.bfloat16, jnp.uint32
    hbm = pl.BlockSpec(memory_space=pltpu.HBM)
    dma = pltpu.SemaphoreType.DMA
    return pl.pallas_call(
        _kernel,
        out_shape=jax.ShapeDtypeStruct(A_q.shape, A_q.dtype),
        in_specs=[hbm] * 11,
        out_specs=hbm,
        scratch_shapes=[
            pltpu.VMEM((S // 2 + 8, D), u32),
            pltpu.VMEM((NL * (S + 16) // 2 + 8, L), u32),
            pltpu.VMEM((S // 2, D), u32),
            pltpu.VMEM((NA * D // 2, UA * T), u32),
            pltpu.VMEM((NF * H, D), u32),
            pltpu.VMEM((NF * H, D), u32),
            pltpu.VMEM((S // 2, D), u32),
            pltpu.VMEM((S // 2, D), u32),
            pltpu.VMEM((S // 2, D), u32),
            *[pltpu.VMEM((S // 2, L), u32)] * NL,
            pltpu.VMEM((NF, S // 2, L), u32),
            pltpu.VMEM((4, NB, T + PX, D), f32),
            pltpu.VMEM((3, NB, T + PG, D), f32),
            pltpu.VMEM((3, NB, T + PK, D), f32),
            pltpu.VMEM((2 * T, D), f32),
            pltpu.VMEM((S, D), f32),
            pltpu.VMEM((NB, T, L), u32),
            pltpu.VMEM((S // 2, D), u32),
            pltpu.VMEM(A_shift_k.shape[::-1], bf16),
            pltpu.VMEM((D,), bf16),
            pltpu.VMEM((F,), bf16),
            pltpu.VMEM((D,), bf16),
            pltpu.VMEM((_DFT.shape[0] // 2, T), u32),
            pltpu.VMEM((NF, 8, L), f32),
            pltpu.VMEM((NL, 8, L), f32),
            pltpu.VMEM(((NF * L - F) // 2, D), u32),
            dma((NA,)), dma((NA,)), dma((NA,)), dma((NA,)), dma((NF // WC,)), dma((1,)), dma((NL + len(LAST),)), dma((5,)),
        ],
        compiler_params=pltpu.CompilerParams(vmem_limit_bytes=110 * 1024 * 1024, disable_bounds_checks=True, flags=FL),
    )(A_q, A_k, A_v, A_shift_k.T, A_ssm_k, A_ssm_D, B_w1.T, B_b1, B_w2, B_b2, jnp.asarray(_DFT, dtype=bf16))
```

```python
import functools
import math

import jax
import jax.numpy as jnp
import numpy as np
import jax.experimental.pallas as pl
import jax.experimental.pallas.tpu as pltpu

T = 128
H = T // 2
L = 128
UA = 2
NP = 2
WC = 2
CQ = 3
PAD = 8
GR, LR = 32, 32
G0, G1, XL = 0.02, 0.76, 6.0
L0, L1 = 0.3, 0.8
KC = (0, 6, 10, 14)
SPLIT = ((14, 16), (11, 14), (8, 11), (0, 8))
M0, MU, FP = 15, 15, 0.55
LAST = ((3, 0, 11), (2, 11, 16))


def _dft_consts():
    k = np.concatenate([np.arange(0, T, 2), T - 1 - np.arange(0, T, 2)])
    n = np.arange(T)
    ang = np.pi * (2 * k[:, None] + 1) * n[None, :] / (2 * T)
    fwd = np.concatenate([np.cos(ang), -np.sin(ang)], 0)
    perm = (n // 16) * 16 + (n % 8) * 2 + (n // 8) % 2
    inv = np.concatenate([np.cos(ang[:H]).T, -np.sin(ang[:H]).T], 1) / T
    r = np.arange(2 * T)
    fwd = fwd[(r // 16) * 8 + r % 8 + (r // 8) % 2 * T]
    return np.concatenate([fwd, fwd[:, perm], inv[0::2], inv[1::2]], 0).astype(np.float32)


_DFT = _dft_consts()
_NT = (((1,), (1,)), ((), ()))


def _kernel(q_hbm, k_hbm, v_hbm, sk_hbm, h_hbm, d_hbm, w1_hbm, b1_hbm, w2_hbm, b2_hbm, f_hbm, o_hbm,
            q_s, k_s, v_s, h_s, w1_s, w2_s, xn0_s, xn1_s, xn2_s, kv0, kv1, kv2, kv3, kv4, act_s,
            xc_s, gc_s, kc_s, hp_s, mlp_s, y_s, o_s, sk_s, d_s, b1_s, b2_s, f_s, b1p_s, b2p_s,
            sq, sk, sv, sh, sw1, sw2, so, sc):
    _, S, D = q_hbm.shape
    F = w1_hbm.shape[0]
    NB = S // T
    NL = D // L
    NF = pl.cdiv(F, L)
    TA = UA * T
    NA = NB // UA
    NW = NF // WC
    f32, bf16, u32 = jnp.float32, jnp.bfloat16, jnp.uint32
    xn_s = (xn0_s, xn1_s, xn2_s)
    kv_s = (kv0, kv1, kv2, kv3, kv4)

    def rows_of(start, n):
        return pl.ds(pl.multiple_of(start, 16), n)

    def lanes(l):
        return pl.ds(pl.multiple_of(l * L, L), L)

    def pk(b, off, n):
        return pl.ds(pl.multiple_of(b * H + off // 2, 8), n // 2)

    def as_bf16(w):
        return pltpu.bitcast(w, bf16)

    def halves(w):
        return (pltpu.bitcast(w << 16, f32), pltpu.bitcast(w & jnp.uint32(0xFFFF0000), f32))

    def q_cp(i):
        return pltpu.make_async_copy(q_hbm.at[0, rows_of(i * TA, TA)],
                                     q_s.bitcast(bf16).at[rows_of(i * TA, TA)], sq.at[i])

    def k_cp(i, n, l):
        return pltpu.make_async_copy(k_hbm.at[0, rows_of(i * TA, n * TA), lanes(l)],
                                     k_s.bitcast(bf16).at[rows_of(i * TA + l * (S + 16) + 16, n * TA)], sk.at[i])

    def v_cp(i, n):
        return pltpu.make_async_copy(v_hbm.at[0, rows_of(i * TA, n * TA)],
                                     v_s.bitcast(bf16).at[rows_of(i * TA, n * TA)], sv.at[i])

    def h_cp(i):
        return pltpu.make_async_copy(h_hbm.at[:, pl.ds(pl.multiple_of(i * TA, TA), TA)],
                                     h_s.bitcast(bf16).at[rows_of(i * D, D)], sh.at[i])

    def w1_cp(c, n):
        return pltpu.make_async_copy(w1_hbm.at[rows_of(c * WC * L, n)],
                                     w1_s.bitcast(bf16).at[rows_of(c * WC * L, n)], sw1.at[c])

    w2_cp = pltpu.make_async_copy(w2_hbm, w2_s.bitcast(bf16).at[pl.ds(0, F)], sw2.at[0])
    small = [pltpu.make_async_copy(a, b, sc.at[j]) for j, (a, b) in enumerate(
        ((b1_hbm, b1_s), (sk_hbm, sk_s), (d_hbm, d_s), (b2_hbm, b2_s), (f_hbm, f_s.bitcast(bf16))))]
    last_w1 = F - (NW - 1) * WC * L

    def group(i, n):
        return ([k_cp(i, n, l) for l in range(NL)] + [v_cp(i, n)] + [h_cp(j) for j in range(i, i + n)]
                + [q_cp(j + NP + 1) for j in range(i, i + n) if j + NP + 1 < NA])

    groups = {0: group(0, 1), 1: group(1, 1), 2: group(2, 2), 4: group(4, NA - 4)}

    small[0].start()
    for i in range(NP):
        q_cp(i).start()
    w1_cp(0, WC * L).start()
    for c in range(1, NW):
        w1_cp(c, WC * L if c < NW - 1 else last_w1).start()
        if c == CQ - 1:
            q_cp(NP).start()
    for cp in small[1:]:
        cp.start()
    for cp in groups[0] + groups[1]:
        cp.start()

    for l in range(NL):
        k_s[pk(0, l * (S + 16), 16), :] = jnp.zeros((8, L), u32)
    hp_s[...] = jnp.zeros(hp_s.shape, f32)
    pad = NF * L - F
    w1_s[pk(0, F, pad), :] = jnp.zeros((pad // 2, D), u32)
    w2_s[pk(0, F, pad), :] = jnp.zeros((pad // 2, D), u32)
    c1 = math.sqrt(2.0 / math.pi)
    c2 = c1 * 0.044715

    def layernorm(b, par, r0, n):
        for j, x in enumerate(halves(q_s[pk(b, r0, n), :])):
            m = jnp.mean(x, axis=-1, keepdims=True)
            xc = x - m
            var = jnp.mean(xc * xc, axis=-1, keepdims=True)
            xn = (xc * jax.lax.rsqrt(var + 1e-5)).astype(bf16)
            for dst in (par, 2):
                xn_s[dst][pk(b, j * H + r0 // 2, n // 2), :] = pltpu.bitcast(xn, u32)

    def mlp1(b, par, n):
        z = jax.lax.dot_general(as_bf16(xn_s[par][pk(b, 0, T), :]), as_bf16(w1_s[pk(n, 0, L), :]), _NT,
                                preferred_element_type=f32)
        a = z + b1p_s[n, 0:1, :]
        t = jnp.tanh(a * (c1 + c2 * (a * a)))
        act_s[n, pk(b, 0, T), :] = pltpu.bitcast((a + a * t).astype(bf16), u32)
        return z

    def gate(b, r0, n, l):
        base = pl.multiple_of(b * H, 8) + (l * (S + 16) + 16 + r0) // 2
        e0, a0 = halves(k_s[pl.ds(base, n // 2), :])
        e1, a1 = halves(k_s[pl.ds(base - 1, n // 2), :])
        _, a2 = halves(k_s[pl.ds(base - 2, n // 2), :])
        t0, t1, t2, t3 = (sk_s[t:t + 1, lanes(l)].astype(f32) for t in range(4))
        ve, va = halves(v_s[pk(b, r0, n), lanes(l)])
        ke = (e0 * t0 + a1 * t1 + e1 * t2 + a2 * t3) * ve
        ka = (a0 * t0 + e0 * t1 + a1 * t2 + e1 * t3) * va
        kv = jnp.concatenate([x[j:j + 8] for j in range(0, n // 2, 8) for x in (ke, ka)], 0)
        kv_s[l][pk(b, r0, n), :] = pltpu.bitcast(kv.astype(bf16), u32)

    def re_im(f):
        return tuple(jnp.concatenate([f[r + o:r + o + 8] for r in range(0, 2 * T, 16)], 0) for o in (0, 8))

    def xdft(b, l):
        xr, xi = re_im(jnp.dot(as_bf16(f_s[T:2 * T, :]), as_bf16(kv_s[l][pk(b, 0, T), :]),
                               preferred_element_type=f32))
        xc_s[0, b, :T, lanes(l)] = xr + xi
        xc_s[1, b, :T, lanes(l)] = xr
        xc_s[2, b, :T, lanes(l)] = xi

    def hpair(i, l, first=True, keep=True):
        prev = hp_s[:, lanes(l)]
        for u in range(UA):
            hb = as_bf16(h_s[pl.ds(pl.multiple_of(i * (D // 2), 8) + l * H, H), u * T:(u + 1) * T])
            hf = jax.lax.dot_general(as_bf16(f_s[0:T, :]), hb, _NT, preferred_element_type=f32)
            hr, hi = re_im(hf)
            pr, pi = re_im(prev)
            gr = jnp.concatenate([hr[:H] - pi[:H], hr[H:] + pi[H:]], 0)
            gi = jnp.concatenate([hi[:H] + pr[:H], hi[H:] - pr[H:]], 0)
            if u == 0 and first:
                dd = d_s[...].astype(f32).reshape(1, D)
                gr = gr + jnp.where(i == 0, dd[:, l * L:(l + 1) * L], 0.0)
            b = i * UA + u
            gc_s[0, b, :T, lanes(l)] = gr
            gc_s[1, b, :T, lanes(l)] = gi - gr
            gc_s[2, b, :T, lanes(l)] = gr + gi
            prev = hf
        if keep:
            hp_s[:, lanes(l)] = prev

    small[0].wait()
    b1 = b1_s[...].astype(f32).reshape(1, F)
    b1p_s[NF - 1] = jnp.zeros((8, L), f32)
    for n in range(NF):
        w = min(L, F - n * L)
        b1p_s[n, 0:1, 0:w] = b1[:, n * L:n * L + w]
    for i in range(NP):
        q_cp(i).wait()
        for u in range(UA):
            layernorm(i * UA + u, u % 2, 0, T)

    def phase_p(c, left):
        @pl.when(c < NW - 1)
        def _():
            w1_cp(c, WC * L).wait()

        @pl.when(c == NW - 1)
        def _():
            w1_cp(NW - 1, last_w1).wait()

        @pl.when(c == CQ)
        def _():
            q_cp(NP).wait()

        for b in (0, 2, 1, 3):
            for n in range(WC):
                z = mlp1(b, b % 2, c * WC + n)
                if b == 1:
                    for r in range(0, H, LR):
                        q_s[S // 2:S // 2 + 8, 0:L] = pltpu.bitcast(z[2 * r:2 * r + 8], u32)
                        layernorm(jnp.where(c < CQ, 0, NP * UA), 0, n * H + r, LR)
        return jnp.minimum(left, NW - c)

    one = jax.lax.fori_loop(0, NW, phase_p, NW)
    for cp in small[1:]:
        cp.wait()
    b2 = b2_s[...].astype(f32).reshape(1, D)
    for l in range(NL):
        b2p_s[l, 0:1, :] = b2[:, l * L:(l + 1) * L]

    def phase_a(i, _):
        im = i + NP
        nxt = jnp.minimum(im + 1, NA - 1)

        @pl.when(i == 1)
        def _():
            for cp in groups[2] + groups[4] + [w2_cp]:
                cp.start()

        for first, cps in groups.items():
            @pl.when(i == first)
            def _(cps=cps):
                for cp in cps:
                    cp.wait()

        nt = UA * NF
        sched = {j: [] for j in range(nt)}
        g_jobs = [(u, l, r) for u in range(UA) for l in range(NL) for r in range(0, T, GR)]
        for j, job in enumerate(g_jobs):
            pos = (G0 + (G1 - G0) * j / len(g_jobs)) * nt
            sched[int(pos)].append((pos % 1, "g", job))
            if j % (len(g_jobs) // NL) == 0:
                sched[int(pos)].append((-1, "h", j // (len(g_jobs) // NL)))
            if job[2] + GR == T:
                sched[int(pos + XL)].append((-1, "x", job[:2]))
        for u in range(UA):
            for j, r in enumerate(range(0, T, LR)):
                pos = (u + L0 + (L1 - L0) * j * LR / T) * NF
                sched[int(pos)].append((pos % 1, "ln", (u, r)))
        for j in range(nt):
            for _, kind, job in sorted(sched[j]):
                if kind == "h":
                    hpair(i, job)
                elif kind == "x":
                    xdft(i * UA + job[0], job[1])
            z = mlp1(im * UA + j // NF, (j // NF) % 2, j % NF)
            for frac, kind, job in sorted(sched[j]):
                r = int(max(frac, 0) * T) // 8 * 8
                hook = pltpu.bitcast(z[r:r + 8], u32)
                if kind == "ln":
                    q_s[S // 2:S // 2 + 8, 0:L] = hook
                    u = job[0] + 1
                    layernorm(im * UA + u if u < UA else nxt * UA, u % 2, job[1], LR)
                elif kind == "g":
                    k_s[pk(0, NL * (S + 16), 16), :] = hook
                    gate(i * UA + job[0], job[2], GR, job[1])
        return 0

    jax.lax.fori_loop(0, NA - NP, phase_a, 0)

    for i in range(NA - NP, NA):
        for l in range(NL):
            hpair(i, l, first=False, keep=i + 1 < NA)
            for u in range(UA):
                gate(i * UA + u, 0, T, l)
            if i > NA - NP:
                for u in range(UA):
                    xdft((i - 1) * UA + u, l)
    for l in range(NL):
        for u in range(UA):
            xdft((NA - 1) * UA + u, l)
    w2_cp.wait()

    def mlp2(b, l, jobs):
        ln = lanes(l)
        acc = None
        done = 0
        for k0, k1 in zip(KC, KC[1:]):
            lhs = jnp.concatenate([as_bf16(act_s[n, pk(b, 0, T), :]) for n in range(k0, k1)], 1)
            part = jnp.dot(lhs, as_bf16(w2_s[pk(k0, 0, (k1 - k0) * L), ln]), preferred_element_type=f32)
            while done < len(jobs) and jobs[done][0] * NF < k1:
                r = max(0, int((jobs[done][0] * NF - k0) / (k1 - k0) * T)) // 8 * 8
                xc_s[3, 0, 0:8, 0:L] = part[r:r + 8]
                jobs[done][1]()
                done += 1
            acc = part if k0 == 0 else acc + part
        x = jnp.concatenate(halves(q_s[pk(b, 0, T), ln]), 0)
        mlp_s[rows_of(b * T, T), ln] = 0.5 * acc + (x + b2p_s[l, 0:1, :])

    def conv_piece(c, rows, ln, o0, o1):
        acc = {}
        for j in range(o1):
            b = xc_s[c, j, rows, ln]
            for o in range(max(o0, j), o1):
                p = gc_s[c, o - j, rows, ln] * b
                acc[o] = p if j == 0 else acc[o] + p
        for o in range(o0, o1):
            kc_s[c, o, rows, ln] = acc[o]

    def fold(b, ln, slot):
        k1 = kc_s[0, b, :T, ln]
        yr, yi = k1 - kc_s[2, b, :T, ln], k1 + kc_s[1, b, :T, ln]
        y = jnp.concatenate([yr[:H] + yr[H:], yi[:H] - yi[H:], yr[:H] - yr[H:], yi[:H] + yi[H:]], 0)
        y_s[slot] = pltpu.bitcast(y.astype(bf16), u32)

    def finish(b, ln, slot):
        y = jnp.concatenate([
            jnp.dot(as_bf16(f_s[2 * T + j * H // 2:2 * T + (j + 1) * H // 2, :]),
                    as_bf16(y_s[slot, j * H:(j + 1) * H, :]), preferred_element_type=f32)
            for j in range(2)], 0)
        out = as_bf16(xn_s[2][pk(b, 0, T), ln]).astype(f32) * y + mlp_s[rows_of(b * T, T), ln]
        o_s[pk(b, 0, T), ln] = pltpu.pack_elementwise([out[:H], out[H:]], packed_dtype=bf16)


    def o_cp(i, l, b, n):
        src = (rows_of(b * T, n * T), lanes(l))
        return pltpu.make_async_copy(o_s.bitcast(bf16).at[src], o_hbm.at[(0,) + src], so.at[i])

    def run_units(first, count, jobs):
        for j in range(count):
            todo = sorted([(p * count - j, job) for p, job in jobs if j <= p * count < j + 1], key=lambda x: x[0])
            mlp2((first + j) % NB, (first + j) // NB, todo)

    def phase_b(l, _, first_stage=False):
        jobs = []
        for b in range(NB):
            if not first_stage:
                jobs.append(functools.partial(fold, b, lanes(l - 1), b))
            jobs += [functools.partial(conv_piece, c, pl.ds(b * 8, 8), lanes(l), o0, o1)
                     for c in range(3) for (o0, o1) in SPLIT]
        jobs = [(p / len(jobs), job) for p, job in enumerate(jobs)]
        if first_stage:
            run_units(0, M0, jobs)
            return 0
        jobs += [((min(b, MU - 1) + FP) / MU, functools.partial(finish, b, lanes(l - 1), b)) for b in range(NB)]
        run_units(M0 + (l - 1) * MU, MU, jobs)
        o_cp(l, l - 1, 0, NB).start()
        return 0

    jax.lax.fori_loop(0, one, functools.partial(phase_b, first_stage=True), 0)
    jax.lax.fori_loop(1, NL, phase_b, 0)

    first = M0 + (NL - 1) * MU
    for i, (n, b0, b1) in enumerate(LAST):
        jobs = [(0.8 * (b - b0) / (b1 - b0), functools.partial(fold, b, lanes(NL - 1), b)) for b in range(b0, b1)]
        jobs += [(0.8 * (b + 1.5 - b0) / (b1 - b0), functools.partial(finish, b, lanes(NL - 1), b))
                 for b in range(b0, b1 - 1)]
        run_units(first, n, jobs)
        finish(b1 - 1, lanes(NL - 1), b1 - 1)
        o_cp(NL + i, NL - 1, b0, b1 - b0).start()
        first += n
    for l in range(1, NL):
        o_cp(l, l - 1, 0, NB).wait()
    for i, (n, b0, b1) in enumerate(LAST):
        o_cp(NL + i, NL - 1, b0, b1 - b0).wait()


@jax.jit
def pallas_parallel_sum__ssm_conv_h3__dense_activation_gelu__prompt_kernel(
    A_q: jax.Array,
    A_k: jax.Array,
    A_v: jax.Array,
    A_shift_k: jax.Array,
    A_ssm_k: jax.Array,
    A_ssm_D: jax.Array,
    B_x: jax.Array,
    B_w1: jax.Array,
    B_b1: jax.Array,
    B_w2: jax.Array,
    B_b2: jax.Array,
):
    del B_x
    _, S, D = A_q.shape
    F = B_w1.shape[1]
    NB = S // T
    NA = NB // UA
    NL = D // L
    NF = pl.cdiv(F, L)
    f32, bf16, u32 = jnp.float32, jnp.bfloat16, jnp.uint32
    hbm = pl.BlockSpec(memory_space=pltpu.HBM)
    dma = pltpu.SemaphoreType.DMA
    return pl.pallas_call(
        _kernel,
        out_shape=jax.ShapeDtypeStruct(A_q.shape, A_q.dtype),
        in_specs=[hbm] * 11,
        out_specs=hbm,
        scratch_shapes=[
            pltpu.VMEM((S // 2 + 8, D), u32),
            pltpu.VMEM((NL * (S + 16) // 2 + 8, L), u32),
            pltpu.VMEM((S // 2, D), u32),
            pltpu.VMEM((NA * D // 2, UA * T), u32),
            pltpu.VMEM((NF * H, D), u32),
            pltpu.VMEM((NF * H, D), u32),
            pltpu.VMEM((S // 2, D), u32),
            pltpu.VMEM((S // 2, D), u32),
            pltpu.VMEM((S // 2, D), u32),
            *[pltpu.VMEM((S // 2, L), u32)] * NL,
            pltpu.VMEM((NF, S // 2, L), u32),
            pltpu.VMEM((4, NB, T + PAD, D), f32),
            pltpu.VMEM((3, NB, T + PAD, D), f32),
            pltpu.VMEM((3, NB, T + PAD, D), f32),
            pltpu.VMEM((2 * T, D), f32),
            pltpu.VMEM((S, D), f32),
            pltpu.VMEM((NB, T, L), u32),
            pltpu.VMEM((S // 2, D), u32),
            pltpu.VMEM(A_shift_k.shape[::-1], bf16),
            pltpu.VMEM((D,), bf16),
            pltpu.VMEM((F,), bf16),
            pltpu.VMEM((D,), bf16),
            pltpu.VMEM((_DFT.shape[0] // 2, T), u32),
            pltpu.VMEM((NF, 8, L), f32),
            pltpu.VMEM((NL, 8, L), f32),
            dma((NA,)), dma((NA,)), dma((NA,)), dma((NA,)), dma((NF // WC,)), dma((1,)), dma((NL + len(LAST),)), dma((5,)),
        ],
        compiler_params=pltpu.CompilerParams(vmem_limit_bytes=110 * 1024 * 1024, disable_bounds_checks=True),
    )(A_q, A_k, A_v, A_shift_k.T, A_ssm_k, A_ssm_D, B_w1.T, B_b1, B_w2, B_b2, jnp.asarray(_DFT, dtype=bf16))
```
